```python
import os as _os
_os.environ.setdefault("JAX_PLATFORMS", "cpu")
import jax
import jax.numpy as jnp

def _softmax(x, axis=-1):
    return jax.nn.softmax(x, axis=axis)
def _gelu(x):
    return jax.nn.gelu(x, approximate=True)
def _silu(x):
    return jax.nn.silu(x)
def _sigmoid(x):
    return jax.nn.sigmoid(x)
def _layernorm(x, axis=-1, eps=1e-5):
    m = jnp.mean(x, axis=axis, keepdims=True)
    v = jnp.var(x, axis=axis, keepdims=True)
    return (x - m) / jnp.sqrt(v + eps)
def _scatter_add(tgt, idx, src, axis=0):
    return tgt.at[idx].add(src)
def _segment_sum(src, seg, n):
    return jax.ops.segment_sum(src, seg, n)
class _Rng:
    def __init__(self, key):
        self._k = key
    def _next(self):
        self._k, sub = jax.random.split(self._k)
        return sub
    def normal(self, shape):
        return jax.random.normal(self._next(), shape, dtype=jnp.bfloat16)
    def randint(self, lo, hi, shape):
        return jax.random.randint(self._next(), shape, lo, hi, dtype=jnp.int32)
    def uniform(self, shape, lo=0.0, hi=1.0):
        return jax.random.uniform(self._next(), shape, jnp.bfloat16, lo, hi)
    def permutation(self, n):
        return jax.random.permutation(self._next(), n)


kernel_name = 'concat_heads__ssm_conv_s4__sliding_local_dilated__prompt'

def setup_inputs():
    _rng = _Rng(jax.random.key(int.from_bytes(__import__("os").urandom(4), "little")))
    _w = (lambda a: (lambda t: t.astype(jnp.bfloat16) if jnp.issubdtype(t.dtype, jnp.floating) else t)(jnp.asarray(a)))
    def _A_setup():
        B, L, D, N = 1, 2048, 640, 192
        A_re = -jnp.exp((lambda *s: _rng.normal(s) * 0.8)(D, N))
        A_im = jnp.pi * (lambda *s: _rng.normal(s) * 0.8)(D, N)
        B_re = (lambda *s: _rng.normal(s) * 0.8)(D, N)
        B_im = (lambda *s: _rng.normal(s) * 0.8)(D, N)
        C_re = (lambda *s: _rng.normal(s) * 0.8)(D, N)
        C_im = (lambda *s: _rng.normal(s) * 0.8)(D, N)
        log_dt = (lambda *s: _rng.normal(s) * 0.8)(D) * 0.5 - 4.0
        Dskip = (lambda *s: _rng.normal(s) * 0.05)(D)
        return {
            "u": _w((lambda *s: _rng.normal(s) * 0.05)(B, L, D)),
            "A_re": _w(A_re),
            "A_im": _w(A_im),
            "B_re": _w(B_re),
            "B_im": _w(B_im),
            "C_re": _w(C_re),
            "C_im": _w(C_im),
            "log_dt": _w(log_dt),
            "Dskip": _w(Dskip),
        }
    _A_in = _A_setup()

    def _B_setup():
        B, S, D = 1, 2048, 640
        return {
            "x": _w((lambda *s: _rng.normal(s) * 0.2)(B, S, D)),
            "wqkv": _w((lambda *s: _rng.normal(s) * 0.2)(D, 3 * D)),
            "wo": _w((lambda *s: _rng.normal(s) * 0.05)(D, D)),
        }
    _B_in = _B_setup()

    return {
        "A_u": _A_in["u"],
        "A_A_re": _A_in["A_re"],
        "A_A_im": _A_in["A_im"],
        "A_B_re": _A_in["B_re"],
        "A_B_im": _A_in["B_im"],
        "A_C_re": _A_in["C_re"],
        "A_C_im": _A_in["C_im"],
        "A_log_dt": _A_in["log_dt"],
        "A_Dskip": _A_in["Dskip"],
        "B_x": _B_in["x"],
        "B_wqkv": _B_in["wqkv"],
        "B_wo": _B_in["wo"],
    }

def reference(A_u, A_A_re, A_A_im, A_B_re, A_B_im, A_C_re, A_C_im, A_log_dt, A_Dskip, B_x, B_wqkv, B_wo):
    def _A_ref(u, A_re, A_im, B_re, B_im, C_re, C_im, log_dt, Dskip):
        Bsz, L, D = u.shape
        dt = jnp.exp(log_dt)[:, None]
        A = A_re + 1j * A_im
        Bc = B_re + 1j * B_im
        Cc = C_re + 1j * C_im
        logdA = dt * A
        dB = dt * Bc
        l = (lambda x, dt: x.astype(dt))(jnp.arange(L), A_re.dtype)
        P = jnp.exp(logdA[:, :, None] * l[None, None, :])
        K = jnp.einsum("dn,dnl,dn->dl", Cc, P, dB).real
        L2 = 2 * L
        Kp = jnp.pad(K, ((0, 0), (0, L)))
        up = (lambda x, *d: x.transpose(*d))(u, 0, 2, 1)
        up = jnp.pad(up, ((0, 0), (0, 0), (0, L)))
        Kf = (lambda x, axes=(-2,-1): jnp.fft.rfft2(x.astype(jnp.float32), axes=axes))(Kp[:, None, :], axes=(-2, -1))
        Uf = (lambda x, axes=(-2,-1): jnp.fft.rfft2(x.astype(jnp.float32), axes=axes))(up[:, :, None, :], axes=(-2, -1))
        Yf = Uf * Kf[None, :, :, :]
        y = (lambda x, s, axes=(-2,-1): jnp.fft.irfft2(x, s=s, axes=axes).astype(jnp.bfloat16))(Yf, (1, L2), axes=(-2, -1))[:, :, 0, :L]
        y = (lambda x, *d: x.transpose(*d))(y, 0, 2, 1) + u * Dskip[None, None, :]
        return y

    def _B_ref(x, wqkv, wo):
        B, S, D = x.shape
        H = 32; Dh = D // H
        W, dil = 8, 2
        qkv = (lambda x, *d: x.transpose(*d))((x @ wqkv).reshape(B, S, 3, H, Dh), 2, 0, 3, 1, 4)
        q, k, v = qkv[0], qkv[1], qkv[2]
        scale = Dh ** -0.5
        pos = jnp.arange(S)
        off = jnp.arange(W) * dil
        idx = pos[:, None] - off[None, :]
        mask = idx >= 0
        idx_c = jnp.where(mask, idx, 0).reshape(-1)
        kg = k[:, :, idx_c, :].reshape(B, H, S, W, Dh)
        vg = v[:, :, idx_c, :].reshape(B, H, S, W, Dh)
        logits = jnp.einsum("bhsd,bhswd->bhsw", q, kg) * scale
        logits = jnp.where(mask[None, None, :, :], logits, -1e9)
        attn = _softmax(logits, axis=-1)
        o = jnp.einsum("bhsw,bhswd->bhsd", attn, vg)
        return (lambda x, *d: x.transpose(*d))(o, 0, 2, 1, 3).reshape(B, S, D) @ wo

    a = _A_ref(A_u, A_A_re, A_A_im, A_B_re, A_B_im, A_C_re, A_C_im, A_log_dt, A_Dskip)
    b = _B_ref(B_x, B_wqkv, B_wo)
    return jnp.concatenate([a, b], axis=-1)
```

```python
import numpy as np
import jax
import jax.numpy as jnp
from jax import lax
import jax.experimental.pallas as pl
import jax.experimental.pallas.tpu as pltpu

L = 2048
D = 640
N = 192
NT = D // 128
NB = L // 128
H, DH, W, DIL = 32, 20, 8, 2
HALO = 16
RB = 128
F32, BF16 = jnp.float32, jnp.bfloat16
SCALE = float(np.float32(DH ** -0.5).astype(jnp.bfloat16))
LOG2E = float(np.log2(np.e))

_HI = ((0, 1, 2, 3), (4, 5, 6, 7), (256, 258, 260, 262), (512, 516, 768, 772),
       (1024, 1280, 1536, 1792))
_KSEG = ((0, 0, 1, None), (1, 1, 1, None), (2, 2, 1, None), (2, 3, 1, 3),
         (3, 4, 3, None), (3, 7, 1, 4), (4, 8, 7, None), (4, 15, 1, 5))


def _bf16_np(a):
    return np.asarray(a, np.float32).astype(jnp.bfloat16)


def _pairs(a):
    bits = a.view(np.uint16).astype(np.uint32)
    return bits[..., 0::2, :] | (bits[..., 1::2, :] << 16)


def _constants():
    j = np.arange(128)
    phi = np.pi * (4 * j[:, None] + 1) * j[None, :] / 256.0
    f = np.concatenate([np.cos(phi), -np.sin(phi)], axis=0)
    g = f.T / 128.0
    where = {}
    for t, hs in enumerate(_HI):
        for n, h in enumerate(hs):
            for m in range(32):
                row = 8 * (m // 2) + 2 * n + m % 2
                where[h + 8 * m] = ((t, row) if t > 1
                                    else (m // 16, 64 * t + row % 64))
    where[L] = (5, 0)
    lag = _bf16_np(np.arange(L)).astype(np.float64).astype(np.int64)
    fk = np.zeros((NB, 256, 128))
    for t, b0, nb, patch in _KSEG:
        for b in range(b0, b0 + nb):
            for p in range(128):
                tt, row = where[int(lag[128 * b + p])]
                if tt == t:
                    assert patch is None or row != 0
                else:
                    assert tt == patch and row == 0
                fk[b, :, row] += f[:, p]
    perm = np.zeros((5, 128, 128))
    for r in range(5):
        perm[r, (DH * (j % H) + 5 * (j // H) + r) % 128, j] = 1.0
    return tuple(_pairs(_bf16_np(a)) for a in (f, g, fk, perm))


_F, _G, _FK, _PERM = _constants()


def _cmul(ar, ai, br, bi):
    return ar * br - ai * bi, ar * bi + ai * br


def _csq(ar, ai):
    return ar * ar - ai * ai, (ar + ar) * ai


def _short_conv(a, b):
    out = []
    for i in range(NB):
        acc = a[0] * b[i]
        for s in range(1, i + 1):
            acc = acc + a[s] * b[i - s]
        out.append(acc)
    return out


def _rows(start, n):
    return pl.ds(start if isinstance(start, int) else pl.multiple_of(start, n), n)


def _load(ref, t, start, rows):
    return pltpu.bitcast(ref.bitcast(jnp.uint32)[t, pl.ds(start // 2 if isinstance(start, int)
                         else pl.multiple_of(start // 2, 8), rows // 2), :], BF16)


def _unpack(x):
    return pltpu.bitcast(x, BF16)


def _kernel(are_hbm, aim_hbm, bre_hbm, bim_hbm, cre_hbm, cim_hbm, ldt_hbm, dsk_hbm,
            u_hbm, x_hbm, wqkv_hbm, wo_hbm, perm_hbm, f_hbm, g_hbm, fk_hbm,
            o_hbm,
            par_s, ldt_s, dsk_s, u_s, x_s, wqkv_s, wo_s, perm_s, f_s, g_s, fk_s,
            tan_s, seed_s, kd_s, kt_s, uh0_s, uh1_s, kh0_s, kh1_s, y0_s, y1_s,
            wp_s, wo32_s, wop_s, qkv0_s, qkv1_s, att_s, oa_s, ob_s, tmp_s,
            uv0_s, uv1_s, prod0_s, prod1_s, flag_s, sems):
    def lanes(c):
        return slice(c * 128, (c + 1) * 128)

    used = []

    def copy(src, dst):
        used.append(None)
        return pltpu.make_async_copy(src, dst, sems.at[len(used) - 1])

    def start(cps):
        for cp in cps:
            cp.start()

    def wait(cps):
        for cp in cps:
            cp.wait()

    cp_first = [copy(ldt_hbm, ldt_s), copy(aim_hbm, par_s.at[0])]
    cp_w = [[copy(wqkv_hbm.at[:, pl.ds(D * p, D)], wqkv_s.at[p])] for p in range(3)]
    cp_x, cp_x2 = [[copy(x_hbm.at[0, rows, lanes(c)], x_s.at[c, rows]) for c in range(NT)]
                   for rows in (pl.ds(0, RB), pl.ds(RB, L - RB))]
    cp_w[0] += [copy(perm_hbm, perm_s)] + cp_x
    cp_par = [copy(src, par_s.at[k + 1])
              for k, src in enumerate((are_hbm, bre_hbm, bim_hbm, cre_hbm, cim_hbm))]
    cp_late = [copy(wo_hbm, wo_s), copy(f_hbm, f_s), copy(g_hbm, g_s), copy(fk_hbm, fk_s),
               copy(dsk_hbm, dsk_s)]
    cp_late += [copy(u_hbm.at[0, :, lanes(c)], u_s.at[c]) for c in range(NT)]
    start(cp_first + cp_w[0] + cp_w[1])
    flag_s[0] = 0

    def spread(order, ties, never):
        started = []
        total = sum(cost for _, cost in order)
        done = 0
        late = None
        for gen, cost in order:
            if gen not in started:
                started.append(gen)
                next(gen)
            tie = ties[done * len(ties) // total]
            done += cost
            if tie is not None and late is not None and CHAIN:
                tie = jnp.where(never, late, tie)

            def after(x, tie=tie):
                if tie is None:
                    return x
                t = jnp.concatenate([tie] * (x.shape[1] // 128), axis=1)
                return jnp.where(never, jnp.concatenate([t] * (x.shape[0] // 8), axis=0), x)

            late = gen.send(after)

    lane = lax.broadcasted_iota(jnp.int32, (8, 128), 1)
    sub = lax.broadcasted_iota(jnp.int32, (8, 128), 0)

    def powers(i, uv):
        low = lane < 64
        top = lax.broadcasted_iota(jnp.int32, (8, 384), 0) < 4

        def pack(re, im):
            return jnp.concatenate(
                [re[:, :128], im[:, :128], jnp.where(low, re[:, 128:], im[:, 128:])], axis=1)

        def wide(x):
            return jnp.concatenate([x[:, :128], x], axis=1)

        def coef(z):
            return z[0] + z[0], z[0] * z[0] + z[1] * z[1]

        def extend(xs, p, q, n):
            p, q = wide(p), wide(q)
            while len(xs) < n:
                xs.append(p * xs[-1] - q * xs[-2])
            return xs

        def put(g, pos, vals, align):
            p = pltpu.pack_elementwise(vals[:2], packed_dtype=BF16)
            q = pltpu.pack_elementwise(vals[2:], packed_dtype=BF16)
            r = pltpu.roll(q, 4, 0)
            uv[g, 0, 8 * pos:8 * pos + 8, :] = jnp.where(top, p, r)
            uv[g, 1, 8 * pos:8 * pos + 8, :] = (
                jnp.where(top, pltpu.roll(p, 4, 0), q) if align else jnp.where(top, r, p))

        late = None
        for g in range(5):
            rows = _rows((i * 5 + g) * 8, 8)
            after = yield late
            z1 = (after(seed_s[0, rows, :]), after(seed_s[1, rows, :]))
            z8 = _csq(*_csq(*_csq(*z1)))
            p8, q8 = coef(z8)
            vs = [pack(jnp.ones((8, 256), F32), jnp.zeros((8, 256), F32)), pack(z8[0], -z8[1])]
            for n in range(4):
                if n:
                    after = yield vs[-4][:, :128]
                    p8 = after(p8)
                extend(vs, p8, q8, 8 * n + 8)
                for k in (2 * n, 2 * n + 1):
                    put(g, k, vs[4 * k:4 * k + 4], True)
            after = yield vs[-4][:, :128]
            z256 = _csq(*_csq(*_csq(*_csq(*_csq(after(z8[0]), after(z8[1]))))))
            w0 = (after(seed_s[2, rows, :]), after(seed_s[3, rows, :]))
            w1 = _cmul(*w0, *z1)
            w256 = _cmul(*w0, *z256)
            w257 = _cmul(*w1, *z256)
            after = yield z256[0][:, :128]
            p1, q1 = coef(z1)
            p1 = after(p1)
            hi = dict(enumerate(extend([pack(*w0), pack(*w1)], p1, q1, 8)))
            hi.update(enumerate(extend([pack(*w256), pack(*w257)], p1, q1, 7), 256))
            for t in range(3):
                put(g, 8 + t, [hi[h] for h in _HI[t]], False)
            after = yield hi[4][:, :128]
            p256, q256 = coef(z256)
            p256 = after(p256)
            for j, n in ((0, 9), (4, 4)):
                for b, val in enumerate(extend([hi[j], hi[256 + j]], p256, q256, n)):
                    hi[256 * b + j] = val
            for t in range(3, 5):
                put(g, 8 + t, [hi[h] for h in _HI[t]], False)
            late = hi[1280][:, :128]
            last = hi[L][:, :128] + jnp.where(low, hi[L][:, 256:], 0.0)
            kd_s[5, rows, :] = jnp.broadcast_to(jnp.sum(last, axis=1, keepdims=True), (8, 128))
        yield late

    def lags(i, g, uv, prod):
        rows = _rows((i * 5 + g) * 8, 8)
        pa, pb = [lax.dot_general(_unpack(uv[g, h, 64:104, :]), _unpack(uv[g, h, 0:64, :]),
                                  (((1,), (1,)), ((), ())), preferred_element_type=F32)
                  for h in range(2)]
        for t in range(5):
            prod[g, 32 * t:32 * t + 8, :] = pa[16 * t:16 * t + 8]
            prod[g, 32 * t + 8:32 * t + 16, :] = pb[16 * t + 8:16 * t + 16]
            prod[g, 32 * t + 16:32 * t + 24, :] = pa[16 * t + 8:16 * t + 16]
            prod[g, 32 * t + 24:32 * t + 32, :] = pb[16 * t:16 * t + 8]
        diag = (lane - 2 * sub) & 6
        for t in range(5):
            m = prod[g, pl.ds(32 * t, 8, stride=2), :]
            for j in range(1, 4):
                pj = prod[g, pl.ds(32 * t + 16 * (j // 2) + j % 2, 8, stride=2), :]
                m = jnp.where(diag == 2 * j, pltpu.roll(pj, 2 * j, 1), m)
            for bit in (1, 2):
                m = jnp.where((sub & bit) != 0, pltpu.roll(m, 128 - 2 * bit, 1), m)
            kd_s[t, rows, :] = m

    def project(i, dst, t):
        xc = jnp.concatenate([_load(x_s, c, i * RB, RB) for c in range(NT)], axis=1)
        res = jnp.dot(xc, _load(wp_s, t, 0, D), preferred_element_type=F32)
        dst[t, HALO:HALO + RB, :] = res
        return [res[8 * k:8 * k + 8] for k in (3, 6, 9, 12, 15)]

    def attend(i, src):
        late = None
        for piece in range(RB // 8):
            r0 = HALO + piece * 8
            after = yield late
            q = [after(src[r, r0:r0 + 8, :]) for r in range(5)]
            logits = []
            for w in range(W):
                rows = slice(r0 - DIL * w, r0 - DIL * w + 8)
                s = q[0] * src[5, rows, :]
                for r in range(1, 5):
                    s = s + q[r] * src[5 + r, rows, :]
                s = s + pltpu.roll(s, 2 * H, 1)
                s = s + pltpu.roll(s, H, 1)
                if piece * 8 < DIL * w:
                    s = jnp.where(i * RB + piece * 8 + sub >= DIL * w, s, -1e9 / SCALE)
                logits.append(s)
            mx = logits[0]
            for v in logits[1:]:
                mx = jnp.maximum(mx, v)
            es = [jnp.exp2((v - mx) * (SCALE * LOG2E)) for v in logits]
            den = es[0]
            for e in es[1:]:
                den = den + e
            inv = 1.0 / den
            outs = []
            for r in range(5):
                acc = es[0] * src[10 + r, r0:r0 + 8, :]
                for w in range(1, W):
                    acc = acc + es[w] * src[10 + r, r0 - DIL * w:r0 - DIL * w + 8, :]
                outs.append(acc * inv)
            if piece % 2:
                out_rows = _rows(i * RB + (piece - 1) * 8, 16)
                for r in range(5):
                    att_s[r, out_rows, :] = jnp.concatenate(
                        [prev[r], outs[r]], axis=0).astype(BF16)
            prev = outs
            late = mx
        yield late

    qkv, uvs, prods = (qkv0_s, qkv1_s), (uv0_s, uv1_s), (prod0_s, prod1_s)

    def stage(i, e):
        for t in range(5, 15):
            qkv[1 - e][t, 0:HALO, :] = qkv[e][t, RB:RB + HALO, :]
        ties = [None] * LEAD
        for t in range(15):
            ties += project(i + 1, qkv[1 - e], t)
            if t % 2 == 1 and t < 10:
                lags(i, t // 2, uvs[e], prods[e])
        pw, at = powers(i + 1, uvs[1 - e]), attend(i, qkv[e])
        order = []
        for n in (4, 2, 4, 2, 4):
            order += [(pw, c) for c in (115, 105, 105, 105, 85, 140, 105)] + [(at, 225)] * n
        spread(order, ties[:-TRAIL], flag_s[0] != 0)

    wait(cp_first)
    dt_row = jnp.exp(ldt_s[...].astype(F32).reshape(1, D)).astype(BF16).astype(F32)

    def angles(c):
        for n in range(0, N, 16):
            after = yield None
            th = after(par_s[0, n:n + 16, lanes(c)].astype(F32)) * dt_row[:, lanes(c)]
            tan_s[c, n:n + 16, :] = jnp.tan(0.5 * th)
        yield None

    def poles(c):
        yield None
        dt = dt_row[:, lanes(c)]
        are, bre, bim, cre, cim = [par_s[k, :, lanes(c)].astype(F32) for k in range(1, 6)]
        t = tan_s[c]
        mag = jnp.exp(dt * are) / (1.0 + t * t)
        vals = (mag * (1.0 - t * t), mag * (t + t)) + _cmul(cre, cim, dt * bre, dt * bim)
        for k, v in enumerate(vals):
            seed_s[k, lanes(c), 0:128] = v[:128].T
            seed_s[k, lanes(c), 128:256] = jnp.concatenate([v[128:], v[128:]], axis=0).T
        yield None

    def reorder(part):
        lane5 = lax.broadcasted_iota(jnp.int32, (D // 2, 128), 1) % 5
        tiles = [pltpu.bitcast(wqkv_s[part, :, lanes(c)], jnp.uint32) for c in range(5)]
        ties = []
        for r in range(5):
            sel = tiles[0]
            for c in range(1, 5):
                sel = jnp.where(lane5 == (r - 128 * c) % 5, tiles[c], sel)
            wp_s[5 * part + r] = jnp.dot(_unpack(sel), _unpack(perm_s[r]),
                                         preferred_element_type=F32).astype(BF16)
        for r in range(5):
            ties += project(0, qkv0_s, 5 * part + r)
        return ties

    for c in range(HEAD[0]):
        spread([(angles(c), 1)] * (N // 16), [None], None)
    for part in range(3):
        wait(cp_w[part] + (cp_par if part == 2 else []))
        start((cp_w[2] + cp_par, cp_x2, [])[part])
        reorder(part)
        for c in range(HEAD[part], HEAD[part + 1]):
            spread([(angles(c), 1)] * (N // 16), [None], None)
    for c in range(NT):
        spread([(poles(c), 1)], [None], None)
    spread([(powers(0, uv0_s), 1)] * 35, [None], None)
    for t in range(5, 15):
        qkv0_s[t, 0:HALO, :] = jnp.broadcast_to(qkv0_s[t, HALO:HALO + 1, :], (HALO, 128))
    wait(cp_x2)
    start(cp_late)

    def tables(c):
        tabs = [kd_s[t, lanes(c), :].T for t in range(6)]
        tabs[:2] = [jnp.concatenate([tabs[0][:64], tabs[1][:64]], axis=0),
                    jnp.concatenate([tabs[0][64:], tabs[1][64:]], axis=0)]
        for t, b0, nb, patch in _KSEG:
            rhs = tabs[t]
            if patch is not None:
                rhs = jnp.concatenate(
                    [jnp.where(sub == 0, tabs[patch][:8], rhs[:8]), rhs[8:]], axis=0)
            rhs = rhs.astype(BF16)
            for b in range(b0, b0 + nb):
                kt_s[c * NB + b] = rhs

    def forward(c, b, uh, kh):
        fu = jnp.dot(_unpack(f_s[...]), _load(u_s, c, b * 128, 128), preferred_element_type=F32)
        uh[b] = fu
        kh[b] = jnp.dot(_unpack(fk_s[b]), _load(kt_s, c * NB + b, 0, 128),
                        preferred_element_type=F32)
        return fu

    def mix(m, uh, kh, y, tmp):
        re = pl.ds(pl.multiple_of(8 * m, 8), 8)
        im = pl.ds(pl.multiple_of(128 + 8 * m, 8), 8)
        for part in range(3):
            if part < 2:
                a = [uh[b, (re, im)[part], :] for b in range(NB)]
            else:
                a = [uh[b, re, :] + uh[b, im, :] for b in range(NB)]
            acc = [None] * NB
            for j in range(NB):
                if j in (0, 3, 7):
                    after = yield None
                if part == 2:
                    k = tmp[0, j]
                else:
                    k = kh[j, (re, im)[part], :]
                k = after(k)
                if part == 0:
                    if j:
                        k = k - kh[j - 1, im, :]
                    tmp[1, j] = k
                elif part == 1:
                    if j:
                        k = k + kh[j - 1, re, :]
                    tmp[0, j] = k + tmp[1, j]
                for i in range(j, NB):
                    p = a[i - j] * k
                    acc[i] = p if j == 0 else acc[i] + p
                if part == 0:
                    tmp[2, j] = acc[j]
                elif part == 1:
                    t = tmp[2, j]
                    y[j, re, :] = t - acc[j]
                    tmp[3, j] = t + acc[j]
                else:
                    y[j, im, :] = acc[j] - tmp[3, j]
        yield None

    def inverse(c, b, y):
        rows = pl.ds(b * 128 if isinstance(b, int) else pl.multiple_of(b * 128, 128), 128)
        res = jnp.dot(_unpack(g_s[...]), y[b].astype(BF16), preferred_element_type=F32)
        oa_s[c, rows, :] = (res + _load(u_s, c, b * 128, 128).astype(F32) * dsk[:, lanes(c)]).astype(BF16)
        return res[-8:]

    def pair(k, carry):
        stage(2 * k, 0)
        stage(2 * k + 1, 1)
        return carry

    nchunk = L // RB
    lax.fori_loop(0, nchunk // 2 - 1, pair, 0)
    tables(0)
    stage(nchunk - 2, 0)

    uh, kh, ys = (uh0_s, uh1_s), (kh0_s, kh1_s), (y0_s, y1_s)
    wait(cp_late)
    dsk = dsk_s[...].astype(F32).reshape(1, D)
    ties = [None] * LEAD
    for b in range(NB):
        fu = forward(0, b, uh0_s, kh0_s)
        ties += [fu[8 * t:8 * t + 8] for t in (0, 8, 16, 24)]
        if b < 5:
            lags(nchunk - 1, b, uv1_s, prod1_s)
    spread([(attend(nchunk - 1, qkv1_s), 1)] * (RB // 8), ties[:-TRAIL], flag_s[0] != 0)
    for c in range(NT):
        wo32_s[c] = wo_s[:, lanes(c)].astype(F32)
    for c in range(NT):
        for r in range(5):
            for j in range(4):
                wop_s[c, 128 * r + H * j:128 * r + H * (j + 1), :] = (
                    wo32_s[c, pl.ds(5 * j + r, H, stride=DH), :].astype(BF16))
    for c in range(1, NT):
        tables(c)

    cp_out = []
    for c in range(NT):
        def body(k, carry, c=c):
            ties = [None] * LAG
            for j in range(UNROLL):
                b = k * UNROLL + j
                rows = pl.ds(pl.multiple_of(b * 128, 128), 128)
                if c + 1 < NT:
                    fu = forward(c + 1, b, uh[(c + 1) % 2], kh[(c + 1) % 2])
                if c > 0:
                    inverse(c - 1, b, ys[(c - 1) % 2])
                ps = [jnp.dot(_load(att_s, r, b * 128, 128), _load(wop_s, c, 128 * r, 128),
                              preferred_element_type=F32) for r in range(5)]
                ob_s[c, rows, :] = (ps[0] + ps[1] + ps[2] + ps[3] + ps[4]).astype(BF16)
                if c + 1 < NT:
                    ties += [fu[8 * t:8 * t + 8] for t in (0, 6, 12, 18, 24, 31)]
                    ties += [ps[4][8 * t:8 * t + 8] for t in (3, 9, 15)]
                else:
                    ties += [ps[0][8 * t:8 * t + 8] for t in (0, 4, 8, 12, 15)]
                    ties += [ps[4][8 * t:8 * t + 8] for t in (3, 7, 11, 15)]
            order = []
            for j in range(UNROLL):
                order += [(mix(k * UNROLL + j, uh[c % 2], kh[c % 2], ys[c % 2],
                               tmp_s.at[j]), 1)] * 9
            spread(order, ties[:-LAG], flag_s[0] != 0)
            return carry

        lax.fori_loop(0, NB // UNROLL, body, 0)
        cps = [copy(ob_s.at[c], o_hbm.at[0, :, lanes(NT + c)])]
        if c > 0:
            cps.append(copy(oa_s.at[c - 1], o_hbm.at[0, :, lanes(c - 1)]))
        start(cps)
        cp_out += cps
    for b in range(NB):
        inverse(NT - 1, b, ys[(NT - 1) % 2])
        if b % 4 == 3:
            rows = pl.ds(128 * (b - 3), 512)
            cp_out.append(copy(oa_s.at[NT - 1, rows], o_hbm.at[0, rows, lanes(NT - 1)]))
            cp_out[-1].start()
    wait(cp_out)


HEAD = (2, 3, 4, 5)
UNROLL = 4
LAG = 3
LEAD = 8
CHAIN = 0
TRAIL = 16


@jax.jit
def pallas_concat_heads__ssm_conv_s4__sliding_local_dilated__prompt_kernel(
    A_u, A_A_re, A_A_im, A_B_re, A_B_im, A_C_re, A_C_im, A_log_dt, A_Dskip, B_x, B_wqkv, B_wo,
):
    hbm = pl.BlockSpec(memory_space=pl.ANY)
    u32 = jnp.uint32
    return pl.pallas_call(
        _kernel,
        out_shape=jax.ShapeDtypeStruct((1, L, 2 * D), BF16),
        in_specs=[hbm] * 16,
        out_specs=hbm,
        scratch_shapes=[
            pltpu.VMEM((6, N, D), BF16),
            pltpu.VMEM((D,), BF16),
            pltpu.VMEM((D,), BF16),
            pltpu.VMEM((NT, L, 128), BF16),
            pltpu.VMEM((NT, L, 128), BF16),
            pltpu.VMEM((3, D, D), BF16),
            pltpu.VMEM((D, D), BF16),
            pltpu.VMEM((5, 64, 128), u32),
            pltpu.VMEM((128, 128), u32),
            pltpu.VMEM((64, 256), u32),
            pltpu.VMEM((NB, 128, 128), u32),
            pltpu.VMEM((NT, N, 128), F32),
            pltpu.VMEM((4, D, 256), F32),
            pltpu.VMEM((6, D, 128), F32),
            pltpu.VMEM((NT * NB, 128, 128), BF16),
        ] + [pltpu.VMEM((NB, 256, 128), F32)] * 6 + [
            pltpu.VMEM((15, D, 128), BF16),
            pltpu.VMEM((NT, D, 128), F32),
            pltpu.VMEM((NT, D, 128), BF16),
            pltpu.VMEM((15, HALO + RB, 128), F32),
            pltpu.VMEM((15, HALO + RB, 128), F32),
            pltpu.VMEM((5, L, 128), BF16),
            pltpu.VMEM((NT, L, 128), BF16),
            pltpu.VMEM((NT, L, 128), BF16),
            pltpu.VMEM((UNROLL, 4, NB, 8, 128), F32),
            pltpu.VMEM((5, 2, 104, 384), u32),
            pltpu.VMEM((5, 2, 104, 384), u32),
            pltpu.VMEM((5, 160, 128), F32),
            pltpu.VMEM((5, 160, 128), F32),
            pltpu.SMEM((1,), jnp.int32),
            pltpu.SemaphoreType.DMA((44,)),
        ],
        compiler_params=pltpu.CompilerParams(vmem_limit_bytes=100 * 1024 * 1024),
    )(A_A_re.T, A_A_im.T, A_B_re.T, A_B_im.T, A_C_re.T, A_C_im.T, A_log_dt, A_Dskip,
      A_u, B_x, B_wqkv, B_wo, _PERM, _F, _G, _FK)
```

```python
import numpy as np
import jax
import jax.numpy as jnp
from jax import lax
import jax.experimental.pallas as pl
import jax.experimental.pallas.tpu as pltpu

L, D, N = 2048, 640, 192
H, DH, W, DIL = 32, 20, 8, 2
NT = D // 128
NB = L // 128
RB = 128
NC = L // RB
NG = 5
HALO = 16
PAD = 8 * NG
SV, SU = 33, 17
GAP = 40
UNROLL = 8
SPLIT = 2
END = 4
F32, BF16, U32 = jnp.float32, jnp.bfloat16, jnp.uint32
SCALE = float(np.float32(DH ** -0.5).astype(BF16))
LOG2E = float(np.log2(np.e))

HEAD = (10, 28, 43, 49, 58)
HCUT = (11, 3)
PM = 64
PT = (3, 6, 9, 12, 15)
LPOS = (1, 3, 5, 7, 9)
LEAD = (6, 5, 8)
TRAIL = (5, 6, 10)
GA = 2
MID = (6, 50)
TF = (0, 2, 5, 8, 11, 14, 17, 20, 23, 26, 29, 31)
LAST = 2
PC = (95, 85, 85, 85, 80, 120, 100)
AC = (70, 140)
CUT = (0, 4, 9, 12)

_HI = ((0, 1, 2, 3), (4, 5, 6, 7), (256, 258, 260, 262), (512, 516, 768, 772),
       (1024, 1280, 1536, 1792))
_KSEG = ((0, 0, 1, None), (1, 1, 1, None), (2, 2, 1, None), (2, 3, 1, 3),
         (3, 4, 3, None), (3, 7, 1, 4), (4, 8, 7, None), (4, 15, 1, 5))
FOLD = 8


def _bf16_np(a):
    return np.asarray(a, np.float32).astype(BF16)


def _pairs(a):
    bits = _bf16_np(a).view(np.uint16).astype(np.uint32)
    return bits[..., 0::2, :] | (bits[..., 1::2, :] << 16)


def _constants():
    j = np.arange(128)
    phi = np.pi * (4 * j[:, None] + 1) * j[None, :] / 256.0
    f = np.concatenate([np.cos(phi), -np.sin(phi)], axis=0)
    g = f.reshape(2, 16, 8, 128).transpose(3, 1, 0, 2).reshape(128, 256) / 128.0
    g = np.stack([g[0::2, :128], g[1::2, :128]])
    where = {L: (5, 0)}
    for t, hs in enumerate(_HI):
        for n, h in enumerate(hs):
            for m in range(32):
                where[h + 8 * m] = ((t, 32 * n + m) if t > 1
                                    else (m // 16, 64 * t + 16 * n + m % 16))
    lag = _bf16_np(np.arange(L)).astype(np.float64).astype(np.int64)
    fk = np.zeros((NB, 256, 128))
    for t, b0, nb, patch in _KSEG:
        for b in range(b0, b0 + nb):
            for p in range(128):
                tile, row = where[int(lag[128 * b + p])]
                assert (tile == t and (patch is None or row)) or (tile == patch and not row)
                fk[b, :, row] += f[:, p]
    for b in range(NB - 1, FOLD, -1):
        fk[b] += np.concatenate([-fk[b - 1, 128:], fk[b - 1, :128]], axis=0)
    perm = np.zeros((5, 128, 128))
    for r in range(5):
        perm[r, (DH * (j % H) + 5 * (j // H) + r) % 128, j] = 1.0
    return tuple(_pairs(a) for a in (perm, f, g, fk))


_PERM, _F, _G, _FK = _constants()


def _cmul(ar, ai, br, bi):
    return ar * br - ai * bi, ar * bi + ai * br


def _square(z, times):
    for _ in range(times):
        z = (z[0] * z[0] - z[1] * z[1], (z[0] + z[0]) * z[1])
    return z


def _lanes(c):
    return slice(c * 128, (c + 1) * 128)


def _rows(start, n):
    return pl.ds(start if isinstance(start, int) else pl.multiple_of(start, n), n)


def _load(ref, t, start, n):
    half = start // 2 if isinstance(start, int) else pl.multiple_of(start // 2, 8)
    return pltpu.bitcast(ref.bitcast(U32)[t, pl.ds(half, n // 2), :], BF16)


def _dot(a, b):
    return jnp.dot(a, b, preferred_element_type=F32)


def _kernel(are_hbm, aim_hbm, bre_hbm, bim_hbm, cre_hbm, cim_hbm, ldt_hbm, dsk_hbm,
            u_hbm, x_hbm, wqkv_hbm, wo_hbm, perm_hbm, f_hbm, g_hbm, fk_hbm,
            o_hbm,
            par_s, ldt_s, dsk_s, u_s, x_s, wqkv_s, wo_s, perm_s, f_s, g_s, fk_s,
            tan_s, seed_s, kd_s, kt_s, wsel_s, wp_s, wo32_s, wop_s, att_s, oa_s, ob_s, tmp_s,
            uh0, uh1, kh0, kh1, y0, y1, qkv0, qkv1, uv0, uv1, prod0, prod1,
            flag_s, sems):
    uhs, khs, ys = (uh0, uh1), (kh0, kh1), (y0, y1)
    qkvs, uvs, prods = (qkv0, qkv1), (uv0, uv1), (prod0, prod1)
    lane = lax.broadcasted_iota(jnp.int32, (8, 128), 1)
    sub = lax.broadcasted_iota(jnp.int32, (8, 128), 0)
    used, started = [], []

    def copy(src, dst):
        used.append(None)
        return pltpu.make_async_copy(src, dst, sems.at[len(used) - 1])

    def start(cps):
        for cp in cps:
            cp.start()

    def wait(cps):
        for cp in cps:
            cp.wait()

    def spread(order, ties=(None,)):
        never = flag_s[0] != 0
        total, done = sum(cost for _, cost in order), 0
        for gen, cost in order:
            if gen not in started:
                started.append(gen)
                next(gen)
            tie = ties[int(done * len(ties) / total)]
            done += cost

            def after(x, tie=tie):
                if tie is None:
                    return x
                t = jnp.concatenate([tie] * (x.shape[1] // 128), axis=1)
                return jnp.where(never, jnp.concatenate([t] * (x.shape[0] // 8), axis=0), x)

            gen.send(after)

    def angles(c):
        for n in range(0, N, 16):
            after = yield
            th = after(par_s[0, n:n + 16, _lanes(c)].astype(F32)) * dt_row[:, _lanes(c)]
            tan_s[c, n:n + 16, :] = jnp.tan(0.5 * th)
        yield

    def poles(c):
        after = yield
        dt = after(jnp.broadcast_to(dt_row[:, _lanes(c)], (8, 128)))
        dt = jnp.concatenate([dt] * (N // 8), axis=0)
        are, bre, bim, cre, cim = [par_s[k, :, _lanes(c)].astype(F32) for k in range(1, 6)]
        t = tan_s[c]
        mag = jnp.exp(dt * are) / (1.0 + t * t)
        vals = (mag * (1.0 - t * t), mag * (t + t)) + _cmul(cre, cim, dt * bre, dt * bim)
        for k, v in enumerate(vals):
            seed_s[k, _lanes(c), 0:128] = v[:128].T
            seed_s[k, _lanes(c), 128:256] = jnp.concatenate([v[128:], v[128:]], axis=0).T
        yield

    def powers(i, uv):
        low = lane < 64

        def parts(re, im):
            return jnp.concatenate(
                [re[:, :128], im[:, :128], jnp.where(low, re[:, 128:], im[:, 128:])], axis=1)

        def coef(z):
            return z[0] + z[0], z[0] * z[0] + z[1] * z[1]

        def extend(xs, p, q, n):
            p, q = [jnp.concatenate([v[:, :128], v], axis=1) for v in (p, q)]
            while len(xs) < n:
                xs.append(p * xs[-1] - q * xs[-2])
            return xs

        def put(g, base, stride, vals):
            for k, v in enumerate(vals):
                for t in range(3):
                    uv[3 * g + t, pl.ds(base + k, 8, stride=stride), :] = v[:, _lanes(t)]

        for g in range(NG):
            rows = _rows((i * NG + g) * 8, 8)
            after = yield
            z1 = (after(seed_s[0, rows, :]), after(seed_s[1, rows, :]))
            z8 = _square(z1, 3)
            p8, q8 = coef(z8)
            vs = [parts(jnp.ones((8, 256), F32), jnp.zeros((8, 256), F32)), parts(z8[0], -z8[1])]
            for n in range(0, 32, 8):
                if n:
                    after = yield
                    p8 = after(p8)
                put(g, n, SV, extend(vs, p8, q8, n + 8)[n:])
            after = yield
            z256 = _square((after(z8[0]), after(z8[1])), 5)
            w0 = (after(seed_s[2, rows, :]), after(seed_s[3, rows, :]))
            w1 = _cmul(*w0, *z1)
            w256 = _cmul(*w0, *z256)
            w257 = _cmul(*w1, *z256)
            after = yield
            p1, q1 = coef(z1)
            p1 = after(p1)
            hi = dict(enumerate(extend([parts(*w0), parts(*w1)], p1, q1, 8)))
            hi.update(enumerate(extend([parts(*w256), parts(*w257)], p1, q1, 7), 256))
            put(g, 8 * SV, SU, [hi[h] for hs in _HI[:3] for h in hs])
            after = yield
            p256, q256 = coef(z256)
            p256 = after(p256)
            for j, n in ((0, 9), (4, 4)):
                for b, val in enumerate(extend([hi[j], hi[256 + j]], p256, q256, n)):
                    hi[256 * b + j] = val
            put(g, 8 * SV + 12, SU, [hi[h] for h in _HI[3]])
            put(g, 8 * (SV + SU), 4, [hi[h] for h in _HI[4]])
            last = hi[L][:, :128] + jnp.where(low, hi[L][:, 256:], 0.0)
            kd_s[5, _rows((i * NG + g) * 8 + PAD, 8), :] = jnp.broadcast_to(
                jnp.sum(last, axis=1, keepdims=True), (8, 128))
        yield

    def power_pieces(i, uv):
        gen = powers(i, uv)
        return [(gen, cost) for cost in PC] * NG

    def lags(g, uv, prod):
        def operand(spans):
            return jnp.concatenate(
                [jnp.concatenate([uv[3 * g + t, a:a + n, :] for a, n in spans], axis=0)
                 for t in range(3)], axis=1).astype(BF16)

        outs = []
        for h in range(2):
            chans = range(4 * h, 4 * h + 4)
            res = lax.dot_general(
                operand([(8 * SV + SU * ch, 16) for ch in chans] + [(8 * (SV + SU) + 16 * h, 16)]),
                operand([(SV * ch, 32) for ch in chans]),
                (((1,), (1,)), ((), ())), preferred_element_type=F32)
            for k in range(4):
                base = 8 + 84 * h + 20 * k
                prod[g, base:base + 16, :] = res[16 * k:16 * k + 16]
                prod[g, base + 16:base + 20, :] = res[64 + 4 * k:68 + 4 * k]
            outs.append(res[-8:])
        return outs + outs[1:]

    def gather(i, g, prod):
        diag = ((lane >> 5) - sub) & 3
        for t in range(-1, 5):
            m = prod[g, pl.ds(8 + 4 * t, 8, stride=21), :]
            for j in range(1, 4):
                pj = prod[g, pl.ds(8 + 4 * t + j, 8, stride=21), :]
                m = jnp.where(diag == j, pltpu.roll(pj, 32 * j, 1), m)
            if t >= 0:
                kd_s[t, _rows((i * NG + g) * 8 + PAD, 8), :] = jnp.where(
                    (lane >> 5) >= (sub & 3), m, prev)
            prev = m

    def reorder(part):
        shift = 3 * lane % 5
        for n in range(0, D // 2, 8):
            tiles = [pltpu.bitcast(wqkv_s[part, 2 * n:2 * n + 16, _lanes(c)], U32)
                     for c in range(5)]
            for bit in (1, 2, 4):
                tiles = [jnp.where((shift & bit) != 0, tiles[(c + bit) % 5], tiles[c])
                         for c in range(5)]
            for r in range(5):
                wsel_s[5 * part + r, n:n + 8, :] = tiles[2 * r % 5]
        ties = []
        for r in range(5):
            res = _dot(pltpu.bitcast(wsel_s[5 * part + r], BF16), pltpu.bitcast(perm_s[r], BF16))
            wp_s[5 * part + r] = res.astype(BF16)
            ties.append([res[128 * k + 120:128 * k + 128] for k in range(5)])
        return [t[k] for k in range(5) for t in ties]

    def project(i, dst, t):
        ties = []
        for n in range(0, RB, PM):
            xc = jnp.concatenate([_load(x_s, c, i * RB + n, PM) for c in range(NT)], axis=1)
            res = _dot(xc, _load(wp_s, t, 0, D))
            dst[t, HALO + n:HALO + n + PM, :] = res
            ties += [res[8 * k - n:8 * k - n + 8] for k in PT if n <= 8 * k < n + PM]
        return ties

    def attend(i, src):
        for piece in range(RB // 8):
            r0 = HALO + piece * 8
            after = yield
            q = [after(src[r, r0:r0 + 8, :]) for r in range(5)]
            sums = []
            for w in range(W):
                rows = slice(r0 - DIL * w, r0 - DIL * w + 8)
                s = q[0] * src[5, rows, :]
                for r in range(1, 5):
                    s = s + q[r] * src[5 + r, rows, :]
                sums.append(s)
            logits = []
            for w, s in enumerate(sums):
                s = ((s + pltpu.roll(s, H, 1))
                     + (pltpu.roll(s, 2 * H, 1) + pltpu.roll(s, 3 * H, 1)))
                if piece * 8 < DIL * w:
                    s = jnp.where(i * RB + piece * 8 + sub >= DIL * w, s, -1e9 / SCALE)
                logits.append(s)
            after = yield
            mx = after(logits[0])
            for v in logits[1:]:
                mx = jnp.maximum(mx, v)
            es = [jnp.exp2((v - mx) * (SCALE * LOG2E)) for v in logits]
            den = es[0]
            for e in es[1:]:
                den = den + e
            inv = 1.0 / den
            outs = []
            for r in range(5):
                acc = es[0] * src[10 + r, r0:r0 + 8, :]
                for w in range(1, W):
                    acc = acc + es[w] * src[10 + r, r0 - DIL * w:r0 - DIL * w + 8, :]
                outs.append(acc * inv)
            if piece % 2:
                for r in range(5):
                    att_s[r, _rows(i * RB + (piece - 1) * 8, 16), :] = jnp.concatenate(
                        [prev[r], outs[r]], axis=0).astype(BF16)
            prev = outs
        yield

    def attention_pieces(i, e):
        gen = attend(i, qkvs[e])
        return [(gen, cost) for cost in AC] * (RB // 8)

    def stage(i, e, z):
        for t in range(5, 15):
            qkvs[1 - e][t, 0:HALO, :] = qkvs[e][t, RB:RB + HALO, :]
        for g in range(NG):
            gather(i - 1, g, prods[1 - e])
        ties = [None] * LEAD[z]
        for t in range(15):
            ties += project(i + 1, qkvs[1 - e], t)
            if t in LPOS:
                ties += lags(LPOS.index(t), uvs[e], prods[e])
        pw, at = power_pieces(i + 1, uvs[1 - e]), attention_pieces(i, e)
        keyed = [((k + 0.5) / len(pw), k, p) for k, p in enumerate(pw)]
        keyed += [((k // GA * GA + 0.5 * GA) / len(at), k, p) for k, p in enumerate(at)]
        spread([p for _, _, p in sorted(keyed, key=lambda t: t[:2])], ties[:-TRAIL[z]])

    def tables(c):
        tabs = [kd_s[t, PAD + 128 * c:PAD + 128 * (c + 1), :].T for t in range(6)]
        tabs[:2] = [jnp.concatenate([tabs[t][32 * n + o:32 * n + o + 16]
                                     for t in range(2) for n in range(4)], axis=0)
                    for o in (0, 16)]
        tabs[0] = jnp.concatenate(
            [tabs[0][:8] + jnp.where(sub == 0, dsk_row[:, _lanes(c)], 0.0), tabs[0][8:]], axis=0)
        for seg, (t, _, _, patch) in enumerate(_KSEG):
            rhs = tabs[t]
            if patch is not None:
                rhs = jnp.concatenate(
                    [jnp.where(sub == 0, tabs[patch][:8], rhs[:8]), rhs[8:]], axis=0)
            kt_s[c * len(_KSEG) + seg] = rhs.astype(BF16)

    def forward(c, b):
        fu = _dot(pltpu.bitcast(f_s[...], BF16), _load(u_s, c, b * 128, 128))
        seg = sum((b >= b0) * 1 for _, b0, _, _ in _KSEG[1:])
        uhs[c % 2][b, 0:256, :] = fu
        khs[c % 2][b, 0:256, :] = _dot(pltpu.bitcast(fk_s[b], BF16),
                                       _load(kt_s, c * len(_KSEG) + seg, 0, 128))
        return fu

    def mix(c, g, half, tmp, other):
        uh, kh, y = uhs[c % 2], khs[c % 2], ys[c % 2]
        re, im = _rows(8 * g + 64 * half, 8), _rows(8 * g + 64 * half + 128, 8)
        for part in range(3):
            def signal(b):
                if part < 2:
                    return uh[b, (re, im)[part], :]
                return uh[b, re, :] + uh[b, im, :]

            def fold(j):
                if part == 2:
                    return tmp[0, j]
                k = kh[j, (re, im)[part], :]
                if 0 < j <= FOLD:
                    k = k + kh[j - 1, re, :] if part else k - kh[j - 1, im, :]
                if part:
                    tmp[0, j] = k + (tmp[4, j] if 0 < j <= FOLD else kh[j, re, :])
                elif 0 < j <= FOLD:
                    tmp[4, j] = k
                return k

            def done(j, v):
                if part == 0:
                    tmp[2, j] = v
                elif part == 1:
                    t = tmp[2, j]
                    tmp[1, j] = t - v
                    tmp[3, j] = t + v
                elif half == 0:
                    tmp[3, j] = v - tmp[3, j]
                else:
                    yr, yi = tmp[1, j], v - tmp[3, j]
                    xr, xi = other[1, j], other[3, j]
                    y[j, _rows(16 * g, 16), :] = jnp.concatenate(
                        [xr + yr, xi + yi], axis=0).astype(BF16)
                    y[j, _rows(16 * g + 128, 16), :] = jnp.concatenate(
                        [xr - yr, xi - yi], axis=0).astype(BF16)

            a = [signal(b) for b in range(NB)]
            acc = [None] * NB
            for j in range(NB):
                k = fold(j)
                if j in CUT:
                    after = yield
                    k = after(k)
                for i in range(j, NB):
                    p = a[i - j] * k
                    acc[i] = p if j == 0 else acc[i] + p
                done(j, acc[j])
        yield

    def inverse(c, b):
        outs = []
        for p in range(2):
            res = _dot(pltpu.bitcast(g_s[p], BF16), _load(ys[c % 2], b, 128 * p, 128))
            outs.append(pltpu.bitcast(res.astype(BF16).astype(F32), U32))
        oa_s.bitcast(U32)[c, _rows(64 * b, 64), :] = (outs[0] >> 16) | outs[1]

    cp_first = [copy(ldt_hbm, ldt_s), copy(aim_hbm, par_s.at[0])]
    cp_w = [[copy(wqkv_hbm.at[:, pl.ds(D * p, D)], wqkv_s.at[p])] for p in range(3)]
    cp_x = [[copy(x_hbm.at[0, rows, _lanes(c)], x_s.at[c, rows]) for c in range(NT)]
            for rows in (pl.ds(0, RB), pl.ds(RB, 2 * RB), pl.ds(3 * RB, L - 3 * RB))]
    cp_w[0] += [copy(perm_hbm, perm_s)] + cp_x[0]
    cp_par = [copy(src, par_s.at[k + 1])
              for k, src in enumerate((are_hbm, bre_hbm, bim_hbm, cre_hbm, cim_hbm))]
    cp_late = [copy(wo_hbm, wo_s), copy(f_hbm, f_s), copy(g_hbm, g_s), copy(fk_hbm, fk_s),
               copy(dsk_hbm, dsk_s)]
    cp_late += [copy(u_hbm.at[0, :, _lanes(c)], u_s.at[c]) for c in range(NT)]
    start(cp_first + cp_w[0])
    flag_s[0] = 0
    for ref in prods:
        ref[...] = jnp.zeros(ref.shape, F32)

    def first(part):
        return [v for r in range(5) for v in project(0, qkv0, 5 * part + r)]

    def cut(ties):
        return [None] * HCUT[0] + ties[:-HCUT[1]]

    wait(cp_first)
    dt_row = jnp.exp(ldt_s[...].astype(F32).reshape(1, D)).astype(BF16).astype(F32)
    ang = [(gen, 400) for gen in map(angles, range(NT)) for _ in range(N // 16)]
    pol = [(poles(c), 400) for c in range(NT)]
    spread(ang[:HEAD[0]])
    start(cp_w[1])
    spread(ang[HEAD[0]:HEAD[1]])
    wait(cp_w[0])
    start(cp_par)
    ties = reorder(0)
    start(cp_w[2])
    spread(ang[HEAD[1]:HEAD[2]], cut(ties + first(0)))
    wait(cp_w[1])
    spread(ang[HEAD[2]:HEAD[3]], cut(reorder(1)))
    wait(cp_par)
    spread(pol[:3] + ang[HEAD[3]:HEAD[4]], cut(first(1)))
    wait(cp_w[2])
    start(cp_x[1])
    spread(pol[3:4] + ang[HEAD[4]:] + pol[4:] + power_pieces(0, uv0), cut(reorder(2) + first(2)))
    for t in range(5, 15):
        qkv0[t, 0:HALO, :] = jnp.broadcast_to(qkv0[t, HALO:HALO + 1, :], (HALO, 128))

    start(cp_x[2])
    wait(cp_x[1])

    def pair(k, carry):
        @pl.when(k == 1)
        def _():
            wait(cp_x[2])
            start(cp_late)

        stage(2 * k, 0, 0)
        stage(2 * k + 1, 1, 1)
        return carry

    lax.fori_loop(0, NC // 2 - 1, pair, 0)
    lax.fori_loop(NC - 2, NC - 1 + flag_s[0], lambda i, carry: (stage(i, 0, 2), carry)[1], 0)

    wait(cp_late)
    dsk_row = dsk_s[...].astype(F32).reshape(1, D)
    tables(0)
    for g in range(NG):
        gather(NC - 2, g, prod0)
    for g in range(NG):
        lags(g, uv1, prod1)
    for g in range(NG):
        gather(NC - 1, g, prod1)
    ties = [None] * MID[0]
    for b in range(NB):
        fu = forward(0, b)
        ties += [fu[8 * t:8 * t + 8] for t in (0, 8, 16, 24)]
    spread(attention_pieces(NC - 1, 1), ties[:MID[1]])
    for c in range(NT):
        wo32_s[c, 0:D, :] = wo_s[:, _lanes(c)].astype(F32)
    for c in range(NT):
        for r in range(5):
            for j in range(4):
                wop_s[c, 128 * r + H * j:128 * r + H * (j + 1), :] = (
                    wo32_s[c, pl.ds(5 * j + r, H, stride=DH), :].astype(BF16))
    for c in range(1, NT):
        tables(c)

    cp_out = []
    for c in range(NT):
        sem = len(used)
        used.extend([None] * (2 * SPLIT * NB // UNROLL))

        def results(k, c=c, sem=sem):
            part = _rows(k * (UNROLL * 128 // SPLIT), UNROLL * 128 // SPLIT)
            return [pltpu.make_async_copy(src.at[part], o_hbm.at[0, part, _lanes(t)],
                                          sems.at[sem + 2 * k + n])
                    for n, (src, t) in enumerate(
                        [(ob_s.at[c], NT + c)] + ([(oa_s.at[c - 1], c - 1)] if c else []))]

        def body(k, carry, c=c, results=results):
            ties = [None] * (0 if c + 1 < NT else LAST)
            for j in range(UNROLL):
                b = k * UNROLL + j
                if c + 1 < NT:
                    fu = forward(c + 1, b)
                    ties += [fu[8 * t:8 * t + 8] for t in TF]
                if c > 0:
                    inverse(c - 1, b)
                if c + 1 < NT:
                    for n in (0, 64):
                        att = [_load(att_s, r, b * 128 + n, 64) for r in range(5)]
                        ob_s[c, _rows(b * 128 + n, 64), :] = _dot(
                            jnp.concatenate(att, axis=1), _load(wop_s, c, 0, D)).astype(BF16)
                else:
                    ps = [_dot(_load(att_s, r, b * 128, 128), _load(wop_s, c, 128 * r, 128))
                          for r in range(5)]
                    ob_s[c, _rows(b * 128, 128), :] = (
                        ps[0] + ps[1] + ps[2] + ps[3] + ps[4]).astype(BF16)
                    ties += [ps[r][8 * t:8 * t + 8] for r in (0, 4) for t in range(0, 16, 3)]
                gen = mix(c, k * (UNROLL // 2) + j // 2, j % 2,
                          tmp_s.at[j], tmp_s.at[j - j % 2])
                spread([(gen, 1)] * 12, ties[12 * j:12 * j + 12])
                if (j + 1) % (UNROLL // SPLIT) == 0:
                    start(results(k * SPLIT + j // (UNROLL // SPLIT)))
            return carry

        lax.fori_loop(0, NB // UNROLL, body, 0)
        for k in range(SPLIT * NB // UNROLL):
            cp_out += results(k)
    for b in range(NB):
        inverse(NT - 1, b)
        if (b + 1) % END == 0:
            rows = pl.ds(128 * (b + 1 - END), 128 * END)
            cp_out.append(copy(oa_s.at[NT - 1, rows], o_hbm.at[0, rows, _lanes(NT - 1)]))
            cp_out[-1].start()
    wait(cp_out)


@jax.jit
def pallas_concat_heads__ssm_conv_s4__sliding_local_dilated__prompt_kernel(
    A_u: jax.Array,
    A_A_re: jax.Array,
    A_A_im: jax.Array,
    A_B_re: jax.Array,
    A_B_im: jax.Array,
    A_C_re: jax.Array,
    A_C_im: jax.Array,
    A_log_dt: jax.Array,
    A_Dskip: jax.Array,
    B_x: jax.Array,
    B_wqkv: jax.Array,
    B_wo: jax.Array,
):
    vm = pltpu.VMEM
    hbm = pl.BlockSpec(memory_space=pl.ANY)
    return pl.pallas_call(
        _kernel,
        out_shape=jax.ShapeDtypeStruct((1, L, 2 * D), BF16),
        in_specs=[hbm] * 16,
        out_specs=hbm,
        scratch_shapes=[
            vm((6, N, D), BF16),
            vm((D,), BF16),
            vm((D,), BF16),
            vm((NT, L, 128), BF16),
            vm((NT, L, 128), BF16),
            vm((3, D, D), BF16),
            vm((D, D), BF16),
            vm(_PERM.shape, U32),
            vm(_F.shape, U32),
            vm(_G.shape, U32),
            vm(_FK.shape, U32),
            vm((NT, N, 128), F32),
            vm((4, D, 256), F32),
            vm((6, PAD + D, 128), F32),
            vm((NT * len(_KSEG), 128, 128), BF16),
            vm((15, D // 2, 128), U32),
            vm((15, D, 128), BF16),
            vm((NT, D + 24, 128), F32),
            vm((NT, D, 128), BF16),
            vm((5, L, 128), BF16),
            vm((NT, L, 128), BF16),
            vm((NT, L, 128), BF16),
            vm((UNROLL, 5, NB + 1, 8, 128), F32),
        ]
        + [vm((NB, 256 + GAP, 128), F32)] * 4
        + [vm((NB, 256 + 2 * GAP, 128), BF16)] * 2
        + [vm((15, HALO + RB, 128), F32)] * 2
        + [vm((3 * NG, 8 * (SV + SU) + 40, 128), F32)] * 2
        + [vm((NG, 200, 128), F32)] * 2
        + [pltpu.SMEM((1,), jnp.int32),
           pltpu.SemaphoreType.DMA((36 + NB // END + NT * 2 * SPLIT * NB // UNROLL,))],
        compiler_params=pltpu.CompilerParams(vmem_limit_bytes=100 * 1024 * 1024),
    )(A_A_re.T, A_A_im.T, A_B_re.T, A_B_im.T, A_C_re.T, A_C_im.T, A_log_dt, A_Dskip,
      A_u, B_x, B_wqkv, B_wo, _PERM, _F, _G, _FK)
```
